```python
import os as _os
_os.environ.setdefault("JAX_PLATFORMS", "cpu")
import jax
import jax.numpy as jnp

def _softmax(x, axis=-1):
    return jax.nn.softmax(x, axis=axis)
def _gelu(x):
    return jax.nn.gelu(x, approximate=True)
def _silu(x):
    return jax.nn.silu(x)
def _sigmoid(x):
    return jax.nn.sigmoid(x)
def _layernorm(x, axis=-1, eps=1e-5):
    m = jnp.mean(x, axis=axis, keepdims=True)
    v = jnp.var(x, axis=axis, keepdims=True)
    return (x - m) / jnp.sqrt(v + eps)
def _scatter_add(tgt, idx, src, axis=0):
    return tgt.at[idx].add(src)
def _segment_sum(src, seg, n):
    return jax.ops.segment_sum(src, seg, n)
class _Rng:
    def __init__(self, key):
        self._k = key
    def _next(self):
        self._k, sub = jax.random.split(self._k)
        return sub
    def normal(self, shape):
        return jax.random.normal(self._next(), shape, dtype=jnp.bfloat16)
    def randint(self, lo, hi, shape):
        return jax.random.randint(self._next(), shape, lo, hi, dtype=jnp.int32)
    def uniform(self, shape, lo=0.0, hi=1.0):
        return jax.random.uniform(self._next(), shape, jnp.bfloat16, lo, hi)
    def permutation(self, n):
        return jax.random.permutation(self._next(), n)


kernel_name = 'standalone__dense_activation_silu__prompt'

def setup_inputs():
    _rng = _Rng(jax.random.key(int.from_bytes(__import__("os").urandom(4), "little")))
    _w = (lambda a: (lambda t: t.astype(jnp.bfloat16) if jnp.issubdtype(t.dtype, jnp.floating) else t)(jnp.asarray(a)))
    B, S, D, F = 1, 2048, 448, 1792
    return {
        "x": _w((lambda *s: _rng.normal(s) * 0.05)(B, S, D)),
        "w1": _w((lambda *s: _rng.normal(s) * 0.05)(D, F) * (D ** -0.5)),
        "w2": _w((lambda *s: _rng.normal(s) * 0.05)(F, D) * (F ** -0.5)),
    }

def reference(x, w1, w2):
    h = jnp.einsum("bsd,df->bsf", x, w1)
    h = _silu(h)
    out = jnp.einsum("bsf,fd->bsd", h, w2)
    return out
```

```python
import jax
import jax.numpy as jnp
import jax.experimental.pallas as pl
import jax.experimental.pallas.tpu as pltpu

T = 128

_LOADS = [("w1", 0, 2), ("x", 0, 2), ("x", 2, 1), ("w1", 2, 2), ("x", 3, 3),
          ("w1", 4, 2), ("x", 6, 4), ("w1", 6, 8), ("x", 10, 6), ("w2", 0, 14)]
_PROGRAM = [
    ("wait", 0), ("T", 0, 2), ("wait", 1), ("mm1", 0, 2, 0, 2),
    ("wait", 2, 3), ("T", 2, 2), ("mm1", 0, 2, 2, 1), ("mm1", 2, 2, 0, 3),
    ("wait", 4, 5), ("T", 4, 2), ("mm1", 0, 4, 3, 3), ("mm1", 4, 2, 0, 6),
    ("wait", 6, 7), ("T", 6, 8), ("mm1", 0, 6, 6, 4), ("mm1", 6, 8, 0, 10),
    ("wait", 8, 9), ("mm1", 0, 14, 10, 6),
    ("mm2", 0, 4), ("mm2", 4, 4), ("mm2", 8, 4), ("mm2", 12, 2), ("mm2", 14, 2),
]
_OUTS = [op[1:] for op in _PROGRAM if op[0] == "mm2"]


def _silu(h):
    hh = h * 0.5
    return hh + hh * jnp.tanh(hh)


def _kernel(x_hbm, w1_hbm, w2_hbm, o_hbm, w1t_v, a_v, sin, sout, *bufs):
    ibuf, obuf = bufs[:len(_LOADS)], bufs[len(_LOADS):]
    src = {"x": x_hbm, "w1": w1_hbm, "w2": w2_hbm}
    n_f = w1_hbm.shape[1] // T
    cps = [pltpu.make_async_copy(src[k].at[:, pl.ds(t0 * T, nt * T)], ibuf[i], sin.at[i])
           for i, (k, t0, nt) in enumerate(_LOADS)]

    def cols(kind, t0, nt):
        parts = []
        for i, (k, a, n) in enumerate(_LOADS):
            lo, hi = max(a, t0), min(a + n, t0 + nt)
            if k == kind and lo < hi:
                parts.append((lo, ibuf[i][:, (lo - a) * T:(hi - a) * T]))
        parts = [p for _, p in sorted(parts, key=lambda q: q[0])]
        return parts[0] if len(parts) == 1 else jnp.concatenate(parts, axis=1)

    for c in cps:
        c.start()
    out_cps = []
    for op in _PROGRAM:
        if op[0] == "wait":
            for i in op[1:]:
                cps[i].wait()
        elif op[0] == "T":
            _, f0, nf = op
            w1t_v[f0 * T:(f0 + nf) * T, :] = cols("w1", f0, nf).T
        elif op[0] == "mm1":
            _, f0, nf, s0, ns = op
            h = jnp.dot(w1t_v[f0 * T:(f0 + nf) * T, :], cols("x", s0, ns),
                        preferred_element_type=jnp.float32)
            a = _silu(h).astype(a_v.dtype)
            for j in range(ns):
                a_v[s0 + j, f0 * T:(f0 + nf) * T, :] = a[:, j * T:(j + 1) * T]
        else:
            _, s0, ns = op
            i = len(out_cps)
            a = jnp.concatenate([a_v[s0 + j] for j in range(ns)], axis=1)
            obuf[i][...] = jnp.dot(cols("w2", 0, n_f), a,
                                   preferred_element_type=jnp.float32).astype(obuf[i].dtype)
            c = pltpu.make_async_copy(obuf[i], o_hbm.at[:, pl.ds(s0 * T, ns * T)], sout.at[i])
            c.start()
            out_cps.append(c)
    for c in out_cps:
        c.wait()


@jax.jit
def pallas_standalone__dense_activation_silu__prompt_kernel(x, w1, w2):
    b, s, d = x.shape
    f = w1.shape[1]
    xt = x.reshape(b * s, d).T
    out_t = pl.pallas_call(
        _kernel,
        in_specs=[pl.BlockSpec(memory_space=pl.ANY)] * 3,
        out_specs=pl.BlockSpec(memory_space=pl.ANY),
        out_shape=jax.ShapeDtypeStruct((d, b * s), x.dtype),
        scratch_shapes=[
            pltpu.VMEM((f, d), w1.dtype),
            pltpu.VMEM((b * s // T, f, T), x.dtype),
            pltpu.SemaphoreType.DMA((len(_LOADS),)),
            pltpu.SemaphoreType.DMA((len(_OUTS),)),
        ] + [pltpu.VMEM((d, nt * T), x.dtype) for (_, _, nt) in _LOADS]
          + [pltpu.VMEM((d, ns * T), x.dtype) for (_, ns) in _OUTS],
        compiler_params=pltpu.CompilerParams(vmem_limit_bytes=64 * 2**20),
    )(xt, w1, w2.T)
    return out_t.T.reshape(b, s, d)
```

```python
import jax
import jax.numpy as jnp
import jax.experimental.pallas as pl
import jax.experimental.pallas.tpu as pltpu

_LANES = 128
_NEG_LOG2_E = -1.4426950408889634


def _silu(h):
    d = jnp.minimum(1.0 + jnp.exp2(h * _NEG_LOG2_E), 3.0e38)
    r = pl.reciprocal(d, approx=True)
    return (h * r) * (2.0 - d * r)


def _dot(a, b):
    return jnp.dot(a, b, preferred_element_type=jnp.float32)


def _ffn_kernel(xt_hbm, w1_hbm, w2t_hbm, yt_hbm,
                w1_ra, w1_rb, x_ra, x_rb, w1_m, x_m, w2t,
                w1t, h_part, act, y_a, y_b, sem):
    D, S = xt_hbm.shape
    F = w1_hbm.shape[1]
    KM = x_m.shape[0]
    KR = D - KM
    FA = w1_ra.shape[1]
    SA = x_ra.shape[1]
    SY = y_a.shape[1]
    T = _LANES

    def load(src, rows, cols, dst, s):
        return pltpu.make_async_copy(
            src.at[pl.ds(*rows), pl.ds(*cols)], dst, sem.at[s])

    rem, main = (KM, KR), (0, KM)
    cp_w1_ra = load(w1_hbm, rem, (0, FA), w1_ra, 0)
    cp_x_ra = load(xt_hbm, rem, (0, SA), x_ra, 1)
    cp_x_rb = load(xt_hbm, rem, (SA, S - SA), x_rb, 2)
    cp_w1_rb = load(w1_hbm, rem, (FA, F - FA), w1_rb, 2)
    cp_w1_m = load(w1_hbm, main, (0, F), w1_m, 0)
    cp_x_m = load(xt_hbm, main, (0, S), x_m, 0)
    cp_w2t = load(w2t_hbm, (0, D), (0, F), w2t, 1)

    def x_rem(s0, s1):
        parts = []
        if s0 < SA:
            parts.append(x_ra[:, s0:min(s1, SA)])
        if s1 > SA:
            parts.append(x_rb[:, max(s0, SA) - SA:s1 - SA])
        return parts[0] if len(parts) == 1 else jnp.concatenate(parts, axis=1)

    def up_rem(f0, f1, s0, s1):
        h_part[f0:f1, s0:s1] = _dot(w1t[f0:f1, KM:D], x_rem(s0, s1))

    out_copies = []

    def down(r0, r1, s0, s1):
        a = jnp.concatenate([act[j] for j in range(s0 // T, s1 // T)], axis=1)
        buf, c0 = (y_a, s0) if s0 < SY else (y_b, s0 - SY)
        buf[r0:r1, c0:c0 + s1 - s0] = _dot(w2t[r0:r1, :], a).astype(buf.dtype)

    def write(r0, r1, s0, s1):
        buf, c0 = (y_a, s0) if s0 < SY else (y_b, s0 - SY)
        cp = pltpu.make_async_copy(
            buf.at[pl.ds(r0, r1 - r0), pl.ds(c0, s1 - s0)],
            yt_hbm.at[pl.ds(r0, r1 - r0), pl.ds(s0, s1 - s0)], sem.at[0])
        cp.start()
        out_copies.append(cp)

    for cp in (cp_w1_ra, cp_x_ra, cp_x_rb, cp_w1_rb):
        cp.start()
    cp_w1_ra.wait()
    cp_w1_m.start()
    cp_x_m.start()
    w1t[0:FA, KM:D] = w1_ra[...].T
    cp_x_ra.wait()
    cp_w2t.start()
    up_rem(0, FA, 0, SA)

    cp_x_rb.wait()
    cp_w1_rb.wait()
    w1t[FA:F, KM:D] = w1_rb[...].T
    FL = F - 2 * T
    up_rem(0, FA, SA, S)
    up_rem(FA, FL, 0, S)
    up_rem(FL, F, 0, S - 4 * T)

    cp_w1_m.wait()
    cp_x_m.wait()
    w1t[:, 0:KM] = w1_m[...].T
    up_rem(FL, F, S - 4 * T, S)
    a = _silu(_dot(w1t[:, 0:KM], x_m[...]) + h_part[...]).astype(act.dtype)
    for j in range(S // T):
        act[j] = a[:, j * T:(j + 1) * T]

    cp_w2t.wait()
    for s0 in range(0, SY, 4 * T):
        down(0, D, s0, s0 + 4 * T)
    write(0, D, 0, SY)
    for piece in ((0, KM, SY, S), (KM, D, SY, S - T), (KM, D, S - T, S)):
        down(*piece)
        write(*piece)
    for cp in out_copies:
        cp.wait()


@jax.jit
def pallas_standalone__dense_activation_silu__prompt_kernel(
    x: jax.Array,
    w1: jax.Array,
    w2: jax.Array,
):
    B, L, D = x.shape
    F = w1.shape[1]
    S = B * L
    T = _LANES
    KM = D // T * T
    FA, SA, SY = 3 * T, 8 * T, S - 4 * T
    dt = x.dtype

    yt = pl.pallas_call(
        _ffn_kernel,
        in_specs=[pl.BlockSpec(memory_space=pl.ANY)] * 3,
        out_specs=pl.BlockSpec(memory_space=pl.ANY),
        out_shape=jax.ShapeDtypeStruct((D, S), dt),
        scratch_shapes=[
            pltpu.VMEM((D - KM, FA), dt),
            pltpu.VMEM((D - KM, F - FA), dt),
            pltpu.VMEM((D - KM, SA), dt),
            pltpu.VMEM((D - KM, S - SA), dt),
            pltpu.VMEM((KM, F), dt),
            pltpu.VMEM((KM, S), dt),
            pltpu.VMEM((D, F), dt),
            pltpu.VMEM((F, D), dt),
            pltpu.VMEM((F, S), jnp.float32),
            pltpu.VMEM((S // T, F, T), dt),
            pltpu.VMEM((D, SY), dt),
            pltpu.VMEM((D, S - SY), dt),
            pltpu.SemaphoreType.DMA((3,)),
        ],
        compiler_params=pltpu.CompilerParams(vmem_limit_bytes=100 * 2**20),
    )(x.reshape(S, D).T, w1, w2.T)
    return yt.T.reshape(B, L, D)
```
